```python
import os as _os
_os.environ.setdefault("JAX_PLATFORMS", "cpu")
import jax
import jax.numpy as jnp

def _softmax(x, axis=-1):
    return jax.nn.softmax(x, axis=axis)
def _gelu(x):
    return jax.nn.gelu(x, approximate=True)
def _silu(x):
    return jax.nn.silu(x)
def _sigmoid(x):
    return jax.nn.sigmoid(x)
def _layernorm(x, axis=-1, eps=1e-5):
    m = jnp.mean(x, axis=axis, keepdims=True)
    v = jnp.var(x, axis=axis, keepdims=True)
    return (x - m) / jnp.sqrt(v + eps)
def _scatter_add(tgt, idx, src, axis=0):
    return tgt.at[idx].add(src)
def _segment_sum(src, seg, n):
    return jax.ops.segment_sum(src, seg, n)
class _Rng:
    def __init__(self, key):
        self._k = key
    def _next(self):
        self._k, sub = jax.random.split(self._k)
        return sub
    def normal(self, shape):
        return jax.random.normal(self._next(), shape, dtype=jnp.bfloat16)
    def randint(self, lo, hi, shape):
        return jax.random.randint(self._next(), shape, lo, hi, dtype=jnp.int32)
    def uniform(self, shape, lo=0.0, hi=1.0):
        return jax.random.uniform(self._next(), shape, jnp.bfloat16, lo, hi)
    def permutation(self, n):
        return jax.random.permutation(self._next(), n)


kernel_name = 'recurrent_scan__softmax_full_mha__glu_gated_glu__prompt'

def setup_inputs():
    _rng = _Rng(jax.random.key(int.from_bytes(__import__("os").urandom(4), "little")))
    _w = (lambda a: (lambda t: t.astype(jnp.bfloat16) if jnp.issubdtype(t.dtype, jnp.floating) else t)(jnp.asarray(a)))
    def _A_setup():
        B, S, D = 1, 2048, 1024
        return {
            "x": _w((lambda *s: _rng.normal(s) * 0.05)(B, S, D)),
            "wqkv": _w((lambda *s: _rng.normal(s) * 0.05)(D, 3 * D)),
            "wo": _w((lambda *s: _rng.normal(s) * 0.05)(D, D)),
        }
    _A_in = _A_setup()

    def _B_setup():
        B, S, D, F = 1, 2048, 1024, 3584
        return {
            "x": _w((lambda *s: _rng.normal(s) * 0.05)(B, S, D)),
            "w_gate": _w((lambda *s: _rng.normal(s) * 0.05)(D, F)),
            "w_up": _w((lambda *s: _rng.normal(s) * 0.05)(D, F)),
            "w_down": _w((lambda *s: _rng.normal(s) * 0.05)(F, D)),
        }
    _B_in = _B_setup()

    return {
        "A_x": _A_in["x"],
        "A_wqkv": _A_in["wqkv"],
        "A_wo": _A_in["wo"],
        "B_x": _B_in["x"],
        "B_w_gate": _B_in["w_gate"],
        "B_w_up": _B_in["w_up"],
        "B_w_down": _B_in["w_down"],
    }

def reference(A_x, A_wqkv, A_wo, B_x, B_w_gate, B_w_up, B_w_down):
    def _A_ref(x, wqkv, wo):
        B, S, D = x.shape
        H = 32; Dh = D // H
        qkv = (lambda x, *d: x.transpose(*d))((x @ wqkv).reshape(B, S, 3, H, Dh), 2, 0, 3, 1, 4)
        q, k, v = qkv[0], qkv[1], qkv[2]
        scale = Dh ** -0.5
        scores = jnp.einsum("bhqd,bhkd->bhqk", q, k) * scale
        p = _softmax(scores, axis=-1)
        o = jnp.einsum("bhqk,bhkd->bhqd", p, v)
        return (lambda x, *d: x.transpose(*d))(o, 0, 2, 1, 3).reshape(B, S, D) @ wo

    def _B_ref(x, w_gate, w_up, w_down):
        g = jnp.einsum("bsd,df->bsf", x, w_gate)
        u = jnp.einsum("bsd,df->bsf", x, w_up)
        h = _sigmoid(g) * u
        return jnp.einsum("bsf,fd->bsd", h, w_down)

    x = A_x
    xn = _layernorm(x, axis=-1)
    s = _A_ref(xn, A_wqkv, A_wo)
    g = _silu(_B_ref(xn, B_w_gate, B_w_up, B_w_down))
    return x + s * g
```

```python
import itertools
import math

import jax
import jax.numpy as jnp
from jax import lax
import jax.experimental.pallas as pl
import jax.experimental.pallas.tpu as pltpu

F32, BF16 = jnp.float32, jnp.bfloat16

S, D, F, DH = 2048, 1024, 3584, 32
TQ = 512
CK = 128
NCK = S // CK
FC = 512
NFC = F // FC
LAG, THROTTLE = 1, 4
MS_WIDE, MS_DOWN, MS_QK, NS_QK = 128, 32, 128, 128
SPAN, NSUB = 56, 1
MP, AP = 8, 8
TAIL = ((128, 256, 64, [(256, 384)]), (256, 384, 64, [(384, 512)]), (384, 480, 48, []), (480, 512, 32, []))
PH = 'pagf'
PROF = False
import contextlib
scope = lambda name: jax.named_scope(name) if PROF else contextlib.nullcontext()

_PRODUCTS = (
    (((1, 0, 0), (1, 1, 1)), ((1, 0, 0), (1, 1, 1))),
    (((1, 1, 0), (1, 1, 1)), ((1, 0, 0),)),
    (((1, 0, 0),), ((1, 0, 1), (-1, 1, 1))),
    (((1, 1, 0), (-1, 0, 0)), ((1, 0, 0), (1, 0, 1))),
    (((1, 1, 1),), ((1, 1, 0), (-1, 0, 0))),
    (((1, 0, 0), (1, 0, 1)), ((1, 1, 1),)),
    (((1, 0, 1), (-1, 1, 1)), ((1, 1, 0), (1, 1, 1))),
)


def _combine(terms, get):
    out = get(terms[0][1], terms[0][2])
    for sign, i, j in terms[1:]:
        out = (lax.add if sign > 0 else lax.sub)(out, get(i, j))
    return out


class _Decoder:
    def __init__(self, emit):
        self.emit, self.m = emit, []

    def push(self, v):
        m = self.m
        m.append(v)
        n = len(m)
        if n == 4:
            self.emit(1, 1, lax.add(lax.add(lax.sub(m[0], m[1]), m[2]), v))
        elif n == 5:
            self.emit(1, 0, lax.add(m[1], v))
            self.t = lax.add(m[0], v)
        elif n == 6:
            self.emit(0, 1, lax.add(m[2], v))
            self.t = lax.sub(self.t, v)
        elif n == 7:
            self.emit(0, 0, lax.add(self.t, v))


def _decode2(product, emit):
    outer = {
        (i, j): _Decoder(lambda a, b, v, i=i, j=j: emit(2 * a + i, 2 * b + j, v))
        for i in range(2) for j in range(2)
    }
    for p in range(7):
        inner = _Decoder(lambda i, j, v: outer[i, j].push(v))
        for q in range(7):
            inner.push(product(7 * p + q))
        yield


def _encode2(side, get, dst, rows, starts):
    for r in starts:
        for p in range(7):
            quad = {
                (i, j): _combine(_PRODUCTS[p][side], lambda a, b: get(r, 2 * a + i, 2 * b + j))
                for i in range(2) for j in range(2)
            }
            for q in range(7):
                v = _combine(_PRODUCTS[q][side], lambda a, b: quad[a, b])
                dst[_rows(r, 8, (7 * p + q) * rows), :] = v.astype(BF16)
            yield


def _interleave(main, n_main, *sides, span=None):
    done, span = [0] * len(sides), span or n_main
    for t in range(n_main):
        next(main)
        for k, (gen, n) in enumerate(sides):
            while done[k] < min(n, -(-n * (t + 1) // span)):
                next(gen)
                done[k] += 1


def _drain(gen):
    for _ in gen:
        pass


def _rows(start, size, offset=0):
    if isinstance(start, int):
        return pl.ds(start + offset, size)
    return pl.ds(pl.multiple_of(lax.add(start, offset), 8), size)


def _pack(v):
    return pltpu.bitcast(v.astype(BF16), jnp.uint32)


def _packed(ref, start, size, cols=slice(None)):
    return pltpu.bitcast(ref[_rows(start, size), cols], BF16)


def _dot(a, b):
    return lax.dot_general(a, b, (((1,), (0,)), ((), ())), preferred_element_type=F32)


def _tree(x, op):
    parts = [lax.slice_in_dim(x, i, i + 8) for i in range(0, x.shape[0], 8)]
    while len(parts) > 1:
        parts = [op(parts[i], parts[i + 1]) for i in range(0, len(parts), 2)]
    return parts[0]


def _sigmoid(x):
    return 0.5 + 0.5 * jnp.tanh(0.5 * x)


def _swap(j):
    return (j % 2) * 2 + j // 2


def _kernel(x_hbm, wqkv_hbm, wo_hbm, wg_hbm, wu_hbm, wd_hbm, out_hbm,
            x_ref, act_ref, xs_ref, w_ref, ws_ref, wd_ref, h_ref, m_ref, acc_ref, sems, idle_sem):
    zero = pl.semaphore_read(idle_sem)
    region = itertools.count(1)

    def block(*streams):
        n = next(region)
        with scope(f"blk{n:02d}"):
            pl.when(zero < n)(lambda: _interleave(*streams))

    def w_copies(left, right, c0, c1):
        return (pltpu.make_async_copy(left.at[:, pl.ds(c0, FC)], w_ref.at[:, 0:FC], sems.at[0]),
                pltpu.make_async_copy(right.at[:, pl.ds(c1, FC)], w_ref.at[:, FC:2 * FC], sems.at[1]))

    def gu_copies(c):
        col = c * FC if isinstance(c, int) else pl.multiple_of(c * FC, FC)
        return w_copies(wg_hbm, wu_hbm, col, col)

    def keep(*refs):
        def body(t, c):
            v = jnp.zeros((16, 128), F32)
            for r in refs:
                for c0 in range(0, r.shape[-1], 128):
                    v += (r[t, 0:16, c0:c0 + 128] if len(r.shape) == 3 else r[_rows(t * 16, 16), c0:c0 + 128]).astype(F32)
            x_ref[_rows(t * 16, 16), 0:128] = v.astype(BF16)
            return c
        lax.fori_loop(0, 4, body, 0)
        cp = pltpu.make_async_copy(x_ref, out_hbm, sems.at[3]); cp.start(); cp.wait()

    def wd_copy(c):
        return pltpu.make_async_copy(wd_hbm.at[_rows(c * FC, FC)], wd_ref, sems.at[10])

    def start(copies):
        for cp in copies:
            cp.start()

    def wait(copies):
        for cp in copies:
            cp.wait()

    def encode_w(starts):
        get = lambda r, i, j: w_ref[_rows(r, 8, i * 256), _swap(j) * 256:(_swap(j) + 1) * 256].astype(F32)
        return _encode2(1, get, ws_ref, 256, starts), 7 * len(starts)

    def encode_act(dst, starts):
        get = lambda r, i, j: jnp.concatenate(
            [act_ref[2 * j + c, _rows(r, 8, i * TQ), :] for c in range(2)], axis=1)
        return _encode2(0, get, dst, TQ, starts), 7 * len(starts)

    def wide_products(src, r0=0, r1=TQ, ms=None, base=0):
        ms = ms or MS_WIDE

        def gen():
            for p in range(49):
                for r in range(r0, r1, ms):
                    m_ref[_rows(base + (p * (TQ + MP) + r), ms), :] = _dot(
                        src[_rows(base + (p * TQ + r), ms), :], ws_ref[_rows(p * 256, 256), :])
                    yield
        return gen(), 49 * (r1 - r0) // ms

    def decode_h(starts):
        def gen():
            for r in starts:
                for c in (0, 128):
                    pending = {}

                    def emit(i, j, v):
                        other = pending.pop((i, j // 2), None)
                        if other is None:
                            pending[i, j // 2] = v
                            return
                        g, u = (v, other) if j % 2 == 0 else (other, v)
                        c0 = (j // 2) * 256 + c
                        h_ref[_rows(r, 8, i * TQ), c0:c0 + 128] = _sigmoid(g) * u

                    yield from _decode2(lambda p: m_ref[_rows(r, 8, p * (TQ + MP)), c:c + 128], emit)
        return gen(), 14 * len(starts)

    def clear_acc(slots):
        def gen():
            for p in slots:
                for r in range(0, TQ, 32):
                    acc_ref[p, r:r + 32] = acc_ref[48, r:r + 32]
                    yield
        return gen(), 16 * len(slots)

    def projection_phase(k_ref, qt_ref, vt_ref, wqk_ref, w1_ref, x1_ref, v_ref):
        x_copies = [
            pltpu.make_async_copy(x_hbm.at[i * TQ:(i + 1) * TQ], x_ref.at[i * TQ:(i + 1) * TQ], sems.at[2 + i])
            for i in range(4)
        ]
        qk_copies = [
            pltpu.make_async_copy(wqkv_hbm.at[:, a:b], wqk_ref.at[:, a:b], sems.at[6 + n])
            for n, (a, b) in enumerate(((0, 512), (512, 1024), (1024, 1536), (1536, 2048)))
        ]
        v_copies = w_copies(wqkv_hbm, wqkv_hbm, 2 * D, 2 * D + FC)
        start([x_copies[0], *qk_copies, *x_copies[1:], *v_copies])

        def layer_norm(i):
            def gen():
                for r in range(i * TQ, (i + 1) * TQ, 8):
                    x = x_ref[r:r + 8, :].astype(F32)
                    xc = x - jnp.mean(x, axis=-1, keepdims=True)
                    var = jnp.mean(xc * xc, axis=-1, keepdims=True)
                    xn = xc * lax.rsqrt(var + 1e-5)
                    for g in range(8):
                        act_ref[g, r:r + 8, :] = xn[:, g * 128:(g + 1) * 128]
                    yield
            return gen(), TQ // 8

        def encode_x1(i):
            def gen():
                for r in range(0, 256, 8):
                    for c in range(2):
                        quad = {
                            (a, b): jnp.concatenate(
                                [act_ref[4 * b + 2 * c + t, _rows(i * TQ + a * 256 + r, 8), :] for t in range(2)],
                                axis=1)
                            for a in range(2) for b in range(2)
                        }
                        for p in range(7):
                            v = _combine(_PRODUCTS[p][0], lambda a, b: quad[a, b])
                            x1_ref[_rows((i * 7 + p) * 256 + r, 8), c * 256:(c + 1) * 256] = v.astype(BF16)
                        yield
            return gen(), 64

        q_scale = DH ** -0.5 * math.log2(math.e)

        summed = [p for p in range(7) if len(_PRODUCTS[p][1]) > 1]

        def encode_qk(cols):
            def gen():
                for u in cols:
                    for r in range(0, 512, 16):
                        get = lambda a, b: wqk_ref[_rows(a * 512 + r, 16), (2 * u + b) * 256:(2 * u + b + 1) * 256]
                        quad = {(a, b): get(a, b).astype(F32) for a in range(2) for b in range(2)}
                        for n, p in enumerate(summed):
                            v = _combine(_PRODUCTS[p][1], lambda a, b: quad[a, b])
                            w1_ref[_rows((u * 5 + n) * 512 + r, 16), :] = v.astype(BF16)
                        yield
            return gen(), 32 * len(cols)

        def qk_slot(i, u, p):
            n = (i % 3 * 4 + u) * 7 + p
            return n // 2, n % 2 * 256

        def qk_products(i):
            for u in range(4):
                for p in range(7):
                    slot, r0 = qk_slot(i, u, p)
                    for c in range(0, 256, NS_QK):
                        for r in range(0, 256, MS_QK):
                            if p in summed:
                                w = w1_ref[_rows((u * 5 + summed.index(p)) * 512, 512), c:c + NS_QK]
                            else:
                                _, a, b = _PRODUCTS[p][1][0]
                                c0 = (2 * u + b) * 256 + c
                                w = wqk_ref[a * 512:(a + 1) * 512, c0:c0 + NS_QK]
                            acc_ref[slot, _rows(r0 + r, MS_QK), c:c + NS_QK] = _dot(
                                x1_ref[_rows((i * 7 + p) * 256 + r, MS_QK), :], w)
                            yield

        def decode_qk(i):
            def gen():
                for u in range(4):
                    for c in range(2):
                        for r0 in range(0, 256, 128):
                            parts = {}
                            for r in range(r0, r0 + 128, 16):
                                def emit(a, b, v):
                                    if u < 2:
                                        parts.setdefault((a, b), []).append(v * q_scale)
                                    else:
                                        g = 4 * (u - 2) + 2 * b + c
                                        k_ref[_rows((g * S + i * TQ + a * 256 + r) // 2, 8), :] = _pack(v)
                                dec = _Decoder(emit)
                                for p in range(7):
                                    slot, row = qk_slot(i, u, p)
                                    dec.push(acc_ref[slot, _rows(row + r, 16), c * 128:(c + 1) * 128])
                                yield
                            for (a, b), v in parts.items():
                                g, c0 = 4 * u + 2 * b + c, a * 256 + r0
                                qt_ref[_rows(i * 512 + g * 64, 64), c0:c0 + 128] = _pack(jnp.concatenate(v, axis=0).T)
                            yield
            return gen(), 16 * 9

        def decode_v():
            def gen():
                for r in range(0, TQ, 8):
                    for c in range(2):
                        def emit(i, j, v):
                            v_ref[2 * _swap(j) + c, _rows(r, 8, i * TQ), :] = v
                        yield from _decode2(lambda p: m_ref[_rows(p * (TQ + MP) + r, 8), c * 128:(c + 1) * 128], emit)
            return gen(), 14 * TQ // 8

        def transpose_v():
            def gen():
                for g in range(8):
                    for r in range(0, S, 256):
                        vt_ref[g * 64:(g + 1) * 64, r:r + 256] = _pack(v_ref[g, r:r + 256, :].T)
                        yield
            return gen(), 8 * S // 256

        n = (256 // MS_QK) * (256 // NS_QK)
        acc_ref[42:49, 0:TQ] = jnp.zeros((7, TQ, 256), F32)
        x_copies[0].wait()
        block(*layer_norm(0))
        qk_copies[0].wait()
        block(*encode_x1(0), encode_qk([0]))
        qk = qk_products(0)
        block(qk, 4 * n)
        qk_copies[1].wait()
        block(qk, 3 * n, encode_qk([1]))
        qk_copies[2].wait()
        block(qk, 7 * n, encode_qk([2]))
        wait([qk_copies[3], x_copies[1]])
        ln = layer_norm(1)[0]
        block(qk, 7 * n, encode_qk([3]), (ln, 32))
        block(qk, 4 * n, (ln, 32))
        block(qk, 3 * n, encode_x1(1))
        wait(x_copies[2:])
        qk = qk_products(1)
        block(qk, 18 * n, layer_norm(2), layer_norm(3))
        wait(v_copies)
        block(qk, 10 * n, encode_x1(2), encode_w(range(0, 256, 8)))
        start(gu_copies(0))
        block(qk_products(2), 28 * n, encode_act(xs_ref, range(0, TQ, 8)), encode_x1(3))
        v, steps = wide_products(xs_ref)
        block(v, steps // 2, decode_qk(0))
        block(v, steps // 2, decode_qk(1), decode_qk(2))
        wait(gu_copies(0))
        block(qk_products(3), 28 * n, decode_v(), encode_w(range(0, 256, 8)))
        start([*gu_copies(1), wd_copy(0)])
        gu, steps = wide_products(xs_ref)
        block(gu, steps // 2, decode_qk(3), clear_acc(range(20, 42)))
        block(gu, steps // 2, transpose_v(), clear_acc(range(20)))
        wait(gu_copies(1))

    def attention_phase(k_ref, qt_ref, vt_ref, ot_ref, state_ref, *s_refs):
        def scores(qb, g, j, c, mx, hist):
            q = _packed(qt_ref, qb * 512 + g * 64 + j * 16, 16)
            q = jnp.concatenate([q if i == j else jnp.zeros_like(q) for i in range(4)], axis=0)
            s = _dot(_packed(k_ref, g * (S // 2) + c * CK // 2, CK // 2), q)
            s_refs[j][c * CK:(c + 1) * CK, :] = s
            for r in range(0, CK, CK // NSUB):
                cm = _tree(s[r:r + CK // NSUB], lax.max)
                mx = cm if c == 0 and r == 0 else jnp.maximum(mx, cm)
                hist.append(mx)
            return mx

        def values(g, j, c, m, acc, l):
            p = jnp.exp2(s_refs[j][c * CK:(c + 1) * CK, :] - m)
            cl = _tree(p, lax.add)
            r = _dot(_packed(vt_ref, g * 64 + j * 16, 16, slice(c * CK, (c + 1) * CK)), p.astype(BF16))
            return (r, cl) if c == 0 else (acc + r, l + cl)

        def steps(it, state, hist, do_scores=True, has_prev=True):
            m = {-2: state[0], -1: state[1]}
            acc, l = state[2:]
            mx = None
            for t in range(4 * NCK if do_scores else NCK + LAG):
                if do_scores:
                    ja, ca = divmod(t, NCK)
                    mx = scores(it // 8, it % 8, ja, ca, mx, hist)
                    if ca == NCK - 1:
                        m[ja] = jnp.broadcast_to(jnp.max(mx, axis=0, keepdims=True), (8, TQ))
                jb, cb = divmod(t - NCK - LAG, NCK)
                if jb >= 0 or has_prev:
                    mb = []
                    for back in range(THROTTLE + NSUB - 1, THROTTLE - 1, -1):
                        v = m[jb] + 0.0 * hist[-back] if len(hist) >= back else m[jb]
                        mb += [v] * (CK // 8 // NSUB)
                    mb = jnp.concatenate(mb, axis=0)
                    src = it - 1 if jb < 0 else it
                    acc, l = values(src % 8, jb % 4, cb, mb, acc, l)
                    if cb == NCK - 1:
                        j = jb % 4
                        ot_ref[j * DH:(j + 1) * DH, :] = acc * (1.0 / jnp.sum(l, axis=0, keepdims=True))
                        if j == 3:
                            act_ref[src % 8, _rows((src // 8) * TQ, TQ), :] = ot_ref[...].T
                state[:] = [m.get(2), m.get(3), acc, l]
                yield

        spans = ((0, 8), (8, 16), (16, 48), (48, 56))

        def iterations(its, first=False, last=False):
            sides = [(decode_h([it * 16, it * 16 + 8]), encode_w([it * 8])) for it in its]

            @pl.when(zero < next(region))
            def _():
                state, hist = [None if first else state_ref[a:b] for a, b in spans], []
                for k, side in enumerate(sides):
                    _interleave(steps(its[k], state, hist, has_prev=k or not first), 4 * NCK, *side, span=SPAN)
                if last:
                    _drain(steps(32, state, [], do_scores=False))
                else:
                    for (a, b), v in zip(spans, state):
                        state_ref[a:b] = v

        def body(t, carry):
            iterations([2 * t, 2 * t + 1])
            return carry

        iterations([0, 1], first=True)
        with scope("att_loop"):
            lax.fori_loop(1, 16, body, 0)
        iterations([], last=True)

    def glu_phase(os_ref, hs_ref, wds_ref):
        def encode_h(starts):
            get = lambda r, i, j: jnp.concatenate(
                [h_ref[_rows(r, 8, i * TQ + a), j * 128:(j + 1) * 128] for a in (0, 256)], axis=1)
            return _encode2(0, get, hs_ref, 256, starts), 7 * len(starts)

        def encode_wd(starts):
            get = lambda r, i, j: wd_ref[_rows(r, 8, i * 128), _swap(3 - j) * 256:(_swap(3 - j) + 1) * 256].astype(F32)
            return _encode2(1, get, wds_ref, 128, starts), 7 * len(starts)

        def down(ms, r0=0, r1=TQ):
            def gen():
                for p in range(49):
                    for r in range(r0, r1, ms):
                        c0 = r // 256 * 128
                        acc_ref[p, r:r + ms] += _dot(hs_ref[_rows(p * 256 + r % 256, ms), c0:c0 + 128],
                                                          wds_ref[_rows(p * 128, 128), :])
                        yield
            return gen(), 49 * (r1 - r0) // ms

        wo_copies = w_copies(wo_hbm, wo_hbm, 0, FC)

        def glu_body(c, carry):
            pl.when(c < NFC - 1)(lambda: start(gu_copies(c + 1)))
            pl.when(c == NFC - 1)(lambda: start(wo_copies))
            wd_copy(c - 1).wait()

            def half(t, carry):
                r0 = jnp.minimum((2 * c - 2 + t) * 48, TQ - 48)
                block(*wide_products(xs_ref, 0, 256, base=t * 256),
                      encode_h([t * 128 + r for r in range(0, 128, 8)]),
                      encode_wd([t * 64 + r for r in range(0, 64, 8)]),
                      encode_act(os_ref, [r0 + r for r in range(0, 48, 8)]))
                return carry
            lax.fori_loop(0, 2, half, 0)
            wd_copy(c).start()
            wait(wo_copies)
            block(*down(MS_DOWN), decode_h(range(0, TQ, 8)), encode_w(range(0, 256, 8)))
            return carry
        if 'p' not in PH and PROF: wd_copy(0).start()
        if 'g' in PH: lax.fori_loop(1, NFC, glu_body, 0)
        if 'f' not in PH:
            wd_copy(0).wait()
            keep(os_ref, hs_ref, wds_ref, ws_ref, xs_ref, h_ref, m_ref, acc_ref, act_ref)
            return

        def decode_gate(r0, r1):
            def gen():
                for r in range(r0, r1, 8):
                    for c in range(2):
                        def emit(i, j, y):
                            act_ref[2 * (3 - j) + c, _rows(r, 8, i * TQ), :] = y * _sigmoid(y)
                        yield from _decode2(lambda p: acc_ref[p, r:r + 8, c * 128:(c + 1) * 128], emit)
            return gen(), 14 * (r1 - r0) // 8

        def finish(r0, r1):
            def gen():
                for r in range(r0, r1, 8):
                    left = {}
                    for c in range(2):
                        def emit(i, j, v):
                            rows, cols = _rows(r, 8, i * TQ), slice(_swap(j) * 256, (_swap(j) + 1) * 256)
                            v = v * act_ref[2 * j + c, rows, :]
                            if c == 0:
                                left[i, j] = v
                                return
                            v = jnp.concatenate([left.pop((i, j)), v], axis=1)
                            x_ref[rows, cols] = (x_ref[rows, cols].astype(F32) + v).astype(BF16)
                        yield from _decode2(lambda p: m_ref[_rows(p * (TQ + MP) + r, 8), c * 128:(c + 1) * 128], emit)
            return gen(), 14 * (r1 - r0) // 8

        out_copies = []

        def write_out(r0, r1):
            for i in range(4):
                rows = slice(i * TQ + r0, i * TQ + r1)
                out_copies.append(pltpu.make_async_copy(x_ref.at[rows], out_hbm.at[rows], sems.at[3]))
                out_copies[-1].start()

        wd_copy(NFC - 1).wait()
        block(*wide_products(os_ref, 0, 128, 64), encode_h(range(0, 256, 8)), encode_wd(range(0, 128, 8)))
        block(*down(128, 0, 256))
        block(*down(64, 256, TQ), decode_gate(0, 256))
        done = 0
        for r0, r1, ms, gate in TAIL:
            block(*wide_products(os_ref, r0, r1, ms), finish(done, r0), *[decode_gate(*g) for g in gate])
            write_out(done, r0)
            done = r0
        block(*finish(done, TQ))
        write_out(done, TQ)
        wait(out_copies)

    def attention_block(*kqv):
        'p' in PH and pl.run_scoped(
            lambda *refs: projection_phase(*kqv, *refs, act_ref),
            pltpu.VMEM((D, 2 * D), BF16),
            pltpu.VMEM((4 * 5 * 512, 256), BF16),
            pltpu.VMEM((4 * 7 * 256, 512), BF16),
        )
        'a' in PH and pl.run_scoped(
            lambda *refs: attention_phase(*kqv, *refs),
            pltpu.VMEM((128, TQ), F32),
            pltpu.VMEM((56, TQ), F32),
            *[pltpu.VMEM((S, TQ), F32)] * 4,
        )
        if 'a' not in PH: keep(*kqv)

    pl.run_scoped(
        attention_block,
        pltpu.VMEM((4 * S, 128), jnp.uint32),
        pltpu.VMEM((2 * D, TQ), jnp.uint32),
        pltpu.VMEM((D // 2, S), jnp.uint32),
    )
    pl.run_scoped(
        glu_phase,
        pltpu.VMEM((49 * TQ, 256), BF16),
        pltpu.VMEM((49 * 256, 256), BF16),
        pltpu.VMEM((49 * 128, 256), BF16),
    )


@jax.jit
def pallas_recurrent_scan__softmax_full_mha__glu_gated_glu__prompt_kernel(
    A_x, A_wqkv, A_wo, B_x, B_w_gate, B_w_up, B_w_down,
):
    del B_x
    hbm = pl.BlockSpec(memory_space=pl.ANY)
    out = pl.pallas_call(
        _kernel,
        out_shape=jax.ShapeDtypeStruct((S, D), A_x.dtype),
        in_specs=[hbm] * 6,
        out_specs=hbm,
        scratch_shapes=[
            pltpu.VMEM((S, D), BF16),
            pltpu.VMEM((8, S + 8, 128), F32),
            pltpu.VMEM((49 * TQ, 256), BF16),
            pltpu.VMEM((D, 2 * FC), BF16),
            pltpu.VMEM((49 * 256, 256), BF16),
            pltpu.VMEM((FC, D), BF16),
            pltpu.VMEM((S, FC), F32),
            pltpu.VMEM((49 * (TQ + MP), 256), F32),
            pltpu.VMEM((49, TQ + AP, 256), F32),
            pltpu.SemaphoreType.DMA((11,)),
            pltpu.SemaphoreType.REGULAR,
        ],
        compiler_params=pltpu.CompilerParams(vmem_limit_bytes=126 * 2**20),
        name="fused_block",
    )(A_x.reshape(S, D), A_wqkv, A_wo, B_w_gate, B_w_up, B_w_down)
    return out.reshape(A_x.shape)
```

```python
import functools
import itertools
import math

import jax
import jax.numpy as jnp
from jax import lax
import jax.experimental.pallas as pl
import jax.experimental.pallas.tpu as pltpu

F32, BF16, U32 = jnp.float32, jnp.bfloat16, jnp.uint32

S, D, F, DH = 2048, 1024, 3584, 32
UNIT = 256
NU = S // UNIT
TQ, CK = 512, 128
NCK = S // CK
TRAIL = NCK + 1
THROTTLE = 4
FC = 512
NFC = F // FC
SLOT = 520
EARLY = 3

_PRODUCTS = (
    (((1, 0, 0), (1, 1, 1)), ((1, 0, 0), (1, 1, 1))),
    (((1, 1, 0), (1, 1, 1)), ((1, 0, 0),)),
    (((1, 0, 0),), ((1, 0, 1), (-1, 1, 1))),
    (((1, 1, 0), (-1, 0, 0)), ((1, 0, 0), (1, 0, 1))),
    (((1, 1, 1),), ((1, 1, 0), (-1, 0, 0))),
    (((1, 0, 0), (1, 0, 1)), ((1, 1, 1),)),
    (((1, 0, 1), (-1, 1, 1)), ((1, 1, 0), (1, 1, 1))),
)
_LHS, _RHS = 0, 1


def _encode(side, levels, get, put, outer=range(7), n=0):
    half = 2 ** (levels - 1)
    for p in outer:
        @functools.cache
        def summed(i, j, terms=_PRODUCTS[p][side]):
            out = get(terms[0][1] * half + i, terms[0][2] * half + j)
            for sign, a, b in terms[1:]:
                out = (lax.add if sign > 0 else lax.sub)(out, get(a * half + i, b * half + j))
            return out

        if levels == 1:
            put(7 * n + p, summed(0, 0))
            yield
            continue
        if levels == 3:
            for i, j in itertools.product(range(4), repeat=2):
                summed(i, j)
                yield
        yield from _encode(side, levels - 1, summed, put, n=7 * n + p)


def _shear(get, by):
    for bit in (1, 2):
        def rows(i, j, get=functools.cache(get), bit=bit):
            return get(i, j) if i & bit else lax.add(get(i, j), lax.mul(get(i | bit, j), by))

        def get(i, j, rows=functools.cache(rows), bit=bit):
            return lax.sub(rows(i, j), lax.mul(rows(i, j ^ bit), by)) if j & bit else rows(i, j)
    return functools.cache(get)


def _encode2(side, get, put):
    get = functools.cache(get)
    sheared = _shear(get, 0.5)
    for fn in (get, sheared):
        for i, j in itertools.product((3, 2, 1, 0), range(4)):
            fn(i, j)
            yield
    yield from _encode(side, 2, sheared, put)


class _Decoder:
    def __init__(self, emit):
        self.emit, self.m = emit, []

    def push(self, v):
        m = self.m
        m.append(v)
        if len(m) == 4:
            self.emit(1, 1, lax.add(lax.add(lax.sub(m[0], m[1]), m[2]), v))
        elif len(m) == 5:
            self.emit(1, 0, lax.add(m[1], v))
            self.t = lax.add(m[0], v)
        elif len(m) == 6:
            self.emit(0, 1, lax.add(m[2], v))
            self.t = lax.sub(self.t, v)
        elif len(m) == 7:
            self.emit(0, 0, lax.add(self.t, v))


def _decode1(product):
    out = {}
    dec = _Decoder(lambda a, b, v: out.update({(a, b): v}))
    for p in range(7):
        dec.push(product(p))
    return out


def _decode2(product, emit):
    sheared = {}
    for i, j in itertools.product(range(2), repeat=2):
        for (a, b), v in _decode1(lambda p: product(4 * p + 2 * i + j)).items():
            sheared[2 * a + i, 2 * b + j] = v
        yield
    get = _shear(lambda i, j: sheared[i, j], -0.5)
    for key in sheared:
        emit(*key, get(*key))
        yield


def _strassen(lhs, rhs, emit):
    dec = _Decoder(emit)
    for q in range(7):
        dec.push(_dot(lhs(q), rhs(q)))
        yield


def _stream(steps):
    return lambda fn: (fn(), steps)


def _chain(*streams):
    return itertools.chain(*[gen for gen, _ in streams]), sum(n for _, n in streams)


def _interleave(main, *sides, slack=0):
    done, span = [0] * len(sides), main[1] - slack
    for t in range(main[1]):
        next(main[0])
        for k, (gen, n) in enumerate(sides):
            while done[k] < min(n, -(-n * (t + 1) // span)):
                next(gen)
                done[k] += 1


def _rows(start, size, offset=0):
    first = lax.add(start, offset)
    return pl.ds(first if isinstance(start, int) else pl.multiple_of(first, 8), size)


def _lanes(tile, n=1):
    return slice(tile * 128, (tile + n) * 128)


def _block_row(r):
    return r + (r >> 6) * (UNIT - 64)


def _words(v, dtype=U32):
    return pltpu.bitcast(v.astype(BF16), dtype)


def _from_words(ref, rows, cols=slice(None)):
    return pltpu.bitcast(ref[rows, cols], BF16)


def _stack_halves(v):
    return lax.concatenate([lax.slice_in_dim(v, c, c + 128, axis=1) for c in (0, 128)], 0)


def _dot(a, b):
    return lax.dot_general(a, b, (((1,), (0,)), ((), ())), preferred_element_type=F32)


def _fold_rows(x, reduce):
    while x.size > 8 * x.shape[-1]:
        x = reduce(x.reshape(-1, 2, 8, x.shape[-1]), axis=1)
    return x.reshape(8, -1)


def _start(copies):
    for cp in copies:
        cp.start()


def _wait(copies):
    for cp in copies:
        cp.wait()


def _kernel(x_hbm, wqkv_hbm, wo_hbm, wg_hbm, wu_hbm, wd_hbm, out_hbm,
            x_ref, act_ref, xs_ref, w_ref, ws_ref, wd_ref, wo_ref, h_ref, m_ref, acc_ref, sems, idle_sem):
    zero = pl.semaphore_read(idle_sem)
    regions = itertools.count(1)

    def region(fn):
        n = next(regions)
        pl.when(zero < n)(fn)

    def stage(*streams):
        region(lambda: _interleave(*streams))

    def gu_copies(c):
        col = c * FC if isinstance(c, int) else pl.multiple_of(c * FC, FC)
        return [pltpu.make_async_copy(src.at[:, pl.ds(col, FC)], w_ref.at[:, n * FC:(n + 1) * FC], sems.at[n])
                for n, src in enumerate((wg_hbm, wu_hbm))]

    def wd_copy(c):
        row = c * FC if isinstance(c, int) else pl.multiple_of(c * FC, FC)
        return pltpu.make_async_copy(wd_hbm.at[pl.ds(row, FC)], wd_ref, sems.at[2])

    def encode_gu(outer, word_rows=range(0, 64, 8)):
        at = [(t, 2 * t) for t in word_rows]

        @_stream(65 * len(outer) * len(at))
        def stream():
            for t, row in at:
                def get(k, j):
                    tile = j // 2 % 2 * 4 + j // 4 * 2 + j % 2
                    return w_ref[_rows(row, 16, k * 128), _lanes(tile)].astype(F32)

                def put(n, v):
                    ws_ref[_rows(t, 8, n * 64), :] = _words(v)
                yield from _encode(_RHS, 3, get, put, outer)
        return stream

    def gate_up(outer, units=range(NU)):
        @_stream(49 * len(outer) * len(units) // 2)
        def stream():
            for p, pair in itertools.product(range(7 * outer[0], 7 * outer[-1] + 7), itertools.batched(units, 2)):
                def lhs(q):
                    return lax.concatenate(
                        [_stack_halves(xs_ref[_rows(((7 * p + q) * NU + u) * 16, 16), :]) for u in pair], 0)

                def emit(a, b, v):
                    for t, u in enumerate(pair):
                        m_ref[_rows(p * SLOT + u * 64 + a * 32, 32), _lanes(b)] = lax.slice_in_dim(
                            v, t * 32, t * 32 + 32)
                yield from _strassen(lhs, lambda q: _from_words(ws_ref, _rows((7 * p + q) * 64, 64)), emit)
        return stream

    def decode_h(starts):
        at = [(r, _block_row(r)) for r in starts]

        @_stream(56 * len(at))
        def stream():
            for (r, row), c in itertools.product(at, range(2)):
                pending = {}

                def emit(i, j, a, b, v):
                    other = pending.pop((a, b, i), None)
                    if other is None:
                        pending[a, b, i] = v
                        return
                    g, u = (other, v) if j else (v, other)
                    h_ref[_rows(row, 8, (2 * a + i) * 64), _lanes(2 * b + c)] = lax.add(u, lax.mul(u, lax.tanh(g)))

                outer = {key: _Decoder(functools.partial(emit, *key))
                         for key in itertools.product(range(2), repeat=2)}
                for p in range(7):
                    for key, v in _decode1(lambda q: m_ref[_rows(r, 8, (7 * p + q) * SLOT), _lanes(c)]).items():
                        outer[key].push(v)
                        yield
        return stream

    def projection_phase(k_ref, qt_ref, vt_ref, wqkv_ref, x2_ref, stat_ref, scale_ref):
        def row_stats(which, first, n_units=1, slot=None):
            base = first * UNIT

            @_stream(n_units * UNIT // 8)
            def stream():
                for r in range(0, n_units * UNIT, 8):
                    rows = _rows(base, 8, r)
                    x = x_ref[rows, :].astype(F32)
                    if which == 0:
                        v = jnp.mean(x, axis=-1, keepdims=True)
                    else:
                        xc = x - jnp.tile(stat_ref[rows, _lanes(0)], (1, 8))
                        v = 0.5 * lax.rsqrt(jnp.mean(xc * xc, axis=-1, keepdims=True) + 1e-5)
                    v = jnp.broadcast_to(v, (8, 128))
                    if slot is None:
                        stat_ref[rows, _lanes(which)] = v
                    else:
                        scale_ref[_rows(slot * UNIT + r, 8), :] = v
                    yield
            return stream

        def normed(row, offset, tile, n, slot=None):
            rows = _rows(row, 8, offset)
            scale = stat_ref[rows, _lanes(1)] if slot is None else scale_ref[_rows(slot * UNIT + offset, 8), :]
            mean, scale = (lax.concatenate([v] * n, 1) for v in (stat_ref[rows, _lanes(0)], scale))
            return lax.mul(lax.sub(x_ref[rows, _lanes(tile, n)].astype(F32), mean), scale)

        def stored(row, offset, tile, n):
            rows = _rows(row + offset, 8)
            return lax.concatenate([act_ref[tile + t, rows, :] for t in range(n)], 1)

        def normalise(u, slot):
            base = u * UNIT

            @_stream(UNIT // 2)
            def stream():
                for r, g in itertools.product(range(0, UNIT, 8), range(0, 8, 2)):
                    v = normed(base, r, g, 2, slot)
                    for t in range(2):
                        act_ref[g + t, _rows(slot * UNIT + r, 8), :] = v[:, _lanes(t)]
                    yield
            return stream

        def encode_x2(slot, xn, row):
            @_stream(8 * 81)
            def stream():
                for r in range(0, 64, 8):
                    def put(n, v):
                        x2_ref[_rows((slot * 49 + n) * 64 + r, 8), :] = v.astype(BF16)
                    yield from _encode2(_LHS, lambda i, k: xn(row, i * 64 + r, 2 * k, 2), put)
            return stream

        def encode_x3(u, xn, row):
            base = u * 16

            @_stream(2 * 7 * 65)
            def stream():
                for r in (0, 8):
                    def get(i, k):
                        return lax.concatenate([xn(row, i * 32 + t + r, k, 1) for t in (0, 16)], 1)

                    def put(n, v):
                        xs_ref[_rows(base, 8, n * NU * 16 + r), :] = v.astype(BF16)
                    yield from _encode(_LHS, 3, get, put)
            return stream

        def encode_qkv(c):
            @_stream(16 * 81)
            def stream():
                for t in range(0, 128, 8):
                    def get(k, j):
                        return wqkv_ref[_rows(k * 256 + 2 * t, 16), _lanes(4 * c + j)].astype(F32)

                    def put(n, v):
                        m_ref[_rows((c // 2 * 49 + n) * 128 + t, 8), _lanes(c % 2)] = _words(v, F32)
                    yield from _encode2(_RHS, get, put)
            return stream

        def product_at(slot, c, n, r, size):
            return _rows(n * SLOT + (slot * 3 + c // 2) * 64 + r, size), _lanes(c % 2)

        def qkv(slots, cols=range(6), outer=range(7)):
            @_stream(7 * len(outer) * len(slots) * len(cols))
            def stream():
                for c, slot, p in itertools.product(cols, slots, outer):
                    def emit(a, b, v):
                        acc_ref[product_at(slot, c, 4 * p + 2 * a + b, 0, 64)] = v
                    yield from _strassen(
                        lambda q: x2_ref[_rows((slot * 49 + 7 * p + q) * 64, 64), :],
                        lambda q: _from_words(m_ref, _rows((c // 2 * 49 + 7 * p + q) * 128, 128), _lanes(c % 2)),
                        emit)
            return stream

        q_scale = 4 * DH ** -0.5 * math.log2(math.e)

        def decode_qkv(slot, cols=range(6)):
            @_stream(8 * 20 * len(cols))
            def stream():
                for c, r in itertools.product(cols, range(0, 64, 8)):
                    def emit(i, j, v):
                        kind, g = divmod(4 * c + j, 8)
                        act_ref[g, _rows((2 + 2 * kind + slot) * UNIT + i * 64 + r, 8), :] = (
                            v if kind else lax.mul(v, q_scale))
                    yield from _decode2(lambda n: acc_ref[product_at(slot, c, n, r, 8)], emit)
            return stream

        def transpose(u, slot):
            q_at, k_at, v_at = (u >> 1) * 512, u * 128, u * 512

            @_stream(48)
            def stream():
                for g, t in itertools.product(range(8), range(2)):
                    get = lambda kind: act_ref[g, _rows((2 + 2 * kind + slot) * UNIT + t * 128, 128), :]
                    qt_ref[_rows(q_at, 64, g * 64), _lanes(2 * slot + t)] = _words(get(0).T)
                    yield
                    k_ref[_rows(k_at, 64, g * S // 2 + t * 64), :] = _words(get(1))
                    yield
                    vt_ref[_rows(v_at, 64, g * 64), _lanes(t)] = _words(get(2).T)
                    yield
            return stream

        @_stream(28 * 12)
        def clear_acc():
            for n, r in itertools.product(range(28), range(0, 384, 32)):
                acc_ref[_rows(n * SLOT + r, 32)] = acc_ref[_rows(n * SLOT + 384 + r % 128, 32)]
                yield

        x_copies = [pltpu.make_async_copy(x_hbm.at[a:b], x_ref.at[a:b], sems.at[3 + n])
                    for n, (a, b) in enumerate(itertools.pairwise((0, UNIT, 2 * UNIT, 4 * UNIT, S)))]
        w_copies = [pltpu.make_async_copy(wqkv_hbm.at[:, _lanes(4 * c, 4)], wqkv_ref.at[:, _lanes(4 * c, 4)],
                                          sems.at[7 + c]) for c in range(6)]
        _start([x_copies[0], w_copies[0]])
        for n in range(28):
            acc_ref[n * SLOT + 384:n * SLOT + 512] = jnp.zeros((128, 256), F32)

        x_copies[0].wait()
        _start([x_copies[1], w_copies[1], w_copies[2]])
        stage(row_stats(0, 0))
        stage(row_stats(1, 0, slot=0))
        stage(normalise(0, 0))
        stage(_chain(encode_x2(0, stored, 0), encode_x3(0, stored, 0)))
        w_copies[0].wait()
        _start([w_copies[3], x_copies[2], *w_copies[4:], x_copies[3], *gu_copies(0)])
        stage(encode_qkv(0))
        x_copies[1].wait()
        stage(row_stats(0, 1))
        stage(qkv([0], [0], range(3)), row_stats(1, 1))
        stage(qkv([0], [0], range(3, 7)), encode_x2(1, normed, UNIT))
        w_copies[1].wait()
        stage(qkv([1], [0]), encode_qkv(1))
        for c, stats in enumerate(([], [], [row_stats(0, 2, 2)], [row_stats(1, 2)]), 1):
            _wait([w_copies[c + 1]] + x_copies[2:3] * (c == 3))
            stage(qkv([0, 1], [c]), _chain(encode_qkv(c + 1), decode_qkv(0, [c - 1])), *stats)
        x_copies[3].wait()
        stage(qkv([0], [5]), _chain(row_stats(0, 4, 4), row_stats(1, 3, slot=1)), decode_qkv(0, [4]))
        stage(qkv([1], [5]), row_stats(1, 4, slot=0),
              _chain(encode_x2(0, normed, 2 * UNIT), normalise(3, 1), decode_qkv(0, [5])))
        _wait(gu_copies(0))

        @pl.loop(1, NU // 2)
        def _(t):
            for slot, other in ((0, 1), (1, 0)):
                u = 2 * t + slot
                ahead = [jnp.minimum(u + n, NU - 1) for n in (1, 2, 3)]
                word = jnp.minimum((u - 2) * 16, 48)
                stage(qkv([slot]), transpose(u - 2, slot), row_stats(1, ahead[2], slot=other),
                      _chain(normalise(ahead[1], slot), encode_x2(other, stored, other * UNIT),
                             encode_x3(ahead[0], stored, other * UNIT), decode_qkv(other),
                             encode_gu(range(EARLY), [word, word + 8])))

        wo_copy = pltpu.make_async_copy(wo_hbm, wo_ref, sems.at[3])
        wo_copy.start()
        stage(gate_up(range(EARLY), (0, 3, 4, 5, 6, 7)),
              _chain(*[encode_x3(u, normed, u * UNIT) for u in (1, 2)], encode_gu([EARLY])))
        stage(_chain(gate_up(range(EARLY), (1, 2)), gate_up([EARLY])),
              _chain(encode_gu(range(EARLY + 1, 7)), decode_qkv(1)))
        _start([*gu_copies(1), wd_copy(0)])
        stage(gate_up(range(EARLY + 1, 7)), _chain(transpose(NU - 2, 0), transpose(NU - 1, 1)), clear_acc)
        _wait([*gu_copies(1), wo_copy])

    def attention_phase(k_ref, qt_ref, vt_ref, ot_ref, state_ref, *s_refs):
        def scores(qb, g, j, c):
            q = _from_words(qt_ref, _rows(qb * 512 + g * 64, 16, j * 16))
            q = lax.concatenate([q if i == j else jnp.zeros_like(q) for i in range(4)], 0)
            s = _dot(_from_words(k_ref, _rows(g * (S // 2), CK // 2, c * CK // 2)), q)
            s_refs[j][c * CK:(c + 1) * CK, :] = s
            return _fold_rows(s, jnp.max)

        def values(g, j, c, m):
            p = jnp.exp2(s_refs[j][c * CK:(c + 1) * CK, :] - jnp.tile(m, (CK // 8, 1)))
            v = _from_words(vt_ref, _rows(g * 64, 16, c // 2 * 512 + j * 16), _lanes(c % 2))
            return _fold_rows(p, jnp.sum), _dot(v, p.astype(BF16))

        def four_heads(it, state, running, do_scores=True, has_prev=True):
            steps = 4 * NCK if do_scores else TRAIL

            @_stream(steps)
            def stream():
                m = {-2: state[0], -1: state[1]}
                acc, l = state[2:]
                place = [((it + back) >> 3, (it + back) & 7) for back in (-1, 0)]
                for t in range(steps):
                    if do_scores:
                        j, c = divmod(t, NCK)
                        part = scores(*place[1], j, c)
                        running.append(part if c == 0 else lax.max(running[-1], part))
                        if c == NCK - 1:
                            m[j] = jnp.broadcast_to(jnp.max(running[-1], axis=0, keepdims=True), (8, TQ))
                    j, c = divmod(t - TRAIL, NCK)
                    if j >= 0 or has_prev:
                        row_max = m[j]
                        if len(running) >= THROTTLE:
                            row_max = row_max + 0.0 * running[-THROTTLE]
                        (qb, g), j = place[j >= 0], j % 4
                        part, o = values(g, j, c, row_max)
                        acc, l = (o, part) if c == 0 else (acc + o, l + part)
                        if c == NCK - 1:
                            ot_ref[j * DH:(j + 1) * DH, :] = acc * (2.0 / jnp.sum(l, axis=0, keepdims=True))
                            if j == 3:
                                act_ref[g, _rows(qb * TQ, TQ), :] = ot_ref[...].T
                    state[:] = [m.get(2), m.get(3), acc, l]
                    yield
            return stream

        spans = list(itertools.pairwise((0, 8, 16, 48, 56)))

        def trip(t, first=False):
            side = _chain(decode_h([t * 32 + r for r in range(0, 32, 8)]), encode_gu(range(EARLY), [(t >> 1) * 8]))

            @region
            def _():
                state, running = [None if first else state_ref[a:b] for a, b in spans], []
                _interleave(_chain(four_heads(2 * t, state, running, has_prev=not first),
                                   four_heads(2 * t + 1, state, running)), side, slack=NCK)
                for (a, b), v in zip(spans, state):
                    state_ref[a:b] = v

        trip(0, first=True)
        pl.loop(1, 16)(trip)
        _interleave(gate_up(range(EARLY)), encode_gu(range(EARLY, 7)),
                    four_heads(32, [state_ref[a:b] for a, b in spans], [], do_scores=False))

    def glu_phase(os_ref, hs_ref, wds_ref, wos_ref):
        def encode_h():
            @_stream(4 * 81 * NU)
            def stream():
                for u, r in itertools.product(range(NU), (0, 8, 32, 40)):
                    def get(i, k):
                        return lax.concatenate(
                            [h_ref[_rows(u * UNIT + i * 64 + r + t, 8), _lanes(k)] for t in (0, 16)], 1)

                    def put(n, v):
                        hs_ref[_rows(n * 256 + u * 32 + r // 32 * 16 + r % 32, 8), :] = v.astype(BF16)
                    yield from _encode2(_LHS, get, put)
            return stream

        def encode_o(starts):
            at = [(r, _block_row(r)) for r in starts]

            @_stream(81 * len(at))
            def stream():
                for r, row in at:
                    def get(i, k):
                        rows = _rows(row, 8, i * 64)
                        return lax.concatenate([act_ref[2 * k + c, rows, :] for c in range(2)], 1)

                    def put(n, v):
                        os_ref[_rows(r, 8, n * 512), :] = v.astype(BF16)
                    yield from _encode2(_LHS, get, put)
            return stream

        def encode_weights(src, dst, column, word_rows):
            depth, at = src.shape[0] // 4, [(t, 2 * t) for t in word_rows]

            @_stream(2 * 81 * len(at))
            def stream():
                for (t, row), c in itertools.product(at, range(2)):
                    def get(k, j):
                        return src[_rows(row, 16, k * depth), _lanes(2 * column(j) + c)].astype(F32)

                    def put(n, v):
                        dst[_rows(t, 8, n * depth // 2), _lanes(c)] = _words(v)
                    yield from _encode2(_RHS, get, put)
            return stream

        def encode_wd():
            return encode_weights(wd_ref, wds_ref, lambda j: 3 - j, range(0, 64, 8))

        def down(r0=0, r1=512):
            @_stream(98 * (r1 - r0) // 32)
            def stream():
                for p, r, c in itertools.product(range(7), range(r0, r1, 32), range(2)):
                    def emit(a, b, v):
                        acc_ref[_rows((4 * p + 2 * a + b) * SLOT + r, 32), _lanes(c)] += v
                    yield from _strassen(
                        lambda q: _stack_halves(hs_ref[_rows((7 * p + q) * 256 + r // 2, 16), :]),
                        lambda q: _from_words(wds_ref, _rows((7 * p + q) * 64, 64), _lanes(c)), emit)
            return stream

        def project(r0, r1, size=32):
            @_stream(98 * (r1 - r0) // size)
            def stream():
                for p, r, c in itertools.product(range(7), range(r0, r1, size), range(2)):
                    def emit(a, b, v):
                        m_ref[_rows((4 * p + 2 * a + b) * SLOT + r, size), _lanes(c)] = v
                    yield from _strassen(
                        lambda q: os_ref[_rows((7 * p + q) * 512 + r, size), :],
                        lambda q: _from_words(wos_ref, _rows((7 * p + q) * 128, 128), _lanes(c)), emit)
            return stream

        def decode_rows(src, emit, r0, r1):
            @_stream(5 * (r1 - r0))
            def stream():
                for r, c in itertools.product(range(r0, r1, 8), range(2)):
                    yield from _decode2(lambda n: src[_rows(n * SLOT + r, 8), _lanes(c)],
                                        lambda i, j, v: emit(_rows(_block_row(r) + i * 64, 8), j, c, v))
            return stream

        def gate(rows, j, c, y):
            half = lax.mul(y, 0.5)
            act_ref[2 * (3 - j) + c, rows, :] = lax.add(half, lax.mul(half, lax.tanh(half)))

        def residual(rows, j, c, s):
            at = rows, _lanes(2 * j + c)
            x_ref[at] = lax.add(x_ref[at].astype(F32), lax.mul(s, act_ref[2 * j + c, rows, :])).astype(BF16)

        @pl.loop(1, NFC)
        def _(c):
            following = gu_copies(jnp.minimum(c + 1, NFC - 1))
            _start(following)
            wd_copy(c - 1).wait()
            word = jnp.minimum((c - 1) * 24, 128 - 24)
            stage(gate_up(range(EARLY, 7)),
                  _chain(encode_h(), encode_wd(),
                         encode_weights(wo_ref, wos_ref, lambda j: j, [word + t for t in (0, 8, 16)])))
            wd_copy(c).start()
            _wait(following)
            stage(down(), _chain(decode_h(range(0, 512, 8)), encode_gu(range(EARLY))))
            row = jnp.minimum((c - 1) * 104, 512 - 104)
            side = _chain(encode_gu(range(EARLY, 7)), encode_o([row + r for r in range(0, 104, 8)]))
            pl.when(c < NFC - 1)(lambda: _interleave(gate_up(range(EARLY)), side))

        out_copies = []

        def write_out(r0, r1):
            for u in range(r0 // 64, -(-r1 // 64)):
                lo, hi = max(r0 - u * 64, 0), min(r1 - u * 64, 64)
                for a, b in [(0, UNIT)] if hi - lo == 64 else [(i + lo, i + hi) for i in range(0, UNIT, 64)]:
                    rows = slice(u * UNIT + a, u * UNIT + b)
                    out_copies.append(pltpu.make_async_copy(x_ref.at[rows], out_hbm.at[rows],
                                                            sems.at[len(out_copies)]))
                    out_copies[-1].start()

        wd_copy(NFC - 1).wait()
        stage(project(0, 192, 64), _chain(encode_h(), encode_wd()))
        stage(down(0, 192))
        stage(down(192, 512), decode_rows(acc_ref, gate, 0, 192))
        done = 0
        for r0, r1, gated in ((192, 320, (192, 320)), (320, 416, (320, 448)), (416, 480, (448, 512)),
                              (480, 512, (0, 0))):
            stage(project(r0, r1), _chain(decode_rows(m_ref, residual, done, r0), decode_rows(acc_ref, gate, *gated)))
            write_out(done, r0)
            done = r0
        stage(decode_rows(m_ref, residual, done, 512))
        write_out(done, 512)
        _wait(out_copies)

    def attention_block(*kqv):
        pl.run_scoped(
            functools.partial(projection_phase, *kqv),
            pltpu.VMEM((D, 3 * D), BF16),
            pltpu.VMEM((2 * 49 * 64, 256), BF16),
            pltpu.VMEM((S, 256), F32),
            pltpu.VMEM((2 * UNIT, 128), F32),
        )
        pl.run_scoped(
            functools.partial(attention_phase, *kqv),
            pltpu.VMEM((4 * DH, TQ), F32),
            pltpu.VMEM((56, TQ), F32),
            *[pltpu.VMEM((S, TQ), F32)] * 4,
        )

    pl.run_scoped(
        attention_block,
        pltpu.VMEM((8 * S // 2, 128), U32),
        pltpu.VMEM((4 * D // 2, TQ), U32),
        pltpu.VMEM((NU * D // 2, UNIT), U32),
    )
    pl.run_scoped(
        glu_phase,
        pltpu.VMEM((49 * 512, 256), BF16),
        pltpu.VMEM((49 * 256, 256), BF16),
        pltpu.VMEM((49 * 64, 256), U32),
        pltpu.VMEM((49 * 128, 256), U32),
    )


@jax.jit
def pallas_recurrent_scan__softmax_full_mha__glu_gated_glu__prompt_kernel(
    A_x: jax.Array,
    A_wqkv: jax.Array,
    A_wo: jax.Array,
    B_x: jax.Array,
    B_w_gate: jax.Array,
    B_w_up: jax.Array,
    B_w_down: jax.Array,
):
    del B_x
    hbm = pl.BlockSpec(memory_space=pl.ANY)
    out = pl.pallas_call(
        _kernel,
        out_shape=jax.ShapeDtypeStruct((S, D), A_x.dtype),
        in_specs=[hbm] * 6,
        out_specs=hbm,
        scratch_shapes=[
            pltpu.VMEM((S, D), BF16),
            pltpu.VMEM((8, S + 8, 128), F32),
            pltpu.VMEM((343 * NU * 16, 256), BF16),
            pltpu.VMEM((D, 2 * FC), BF16),
            pltpu.VMEM((343 * 64, 128), U32),
            pltpu.VMEM((FC, D), BF16),
            pltpu.VMEM((D, D), BF16),
            pltpu.VMEM((S, FC), F32),
            pltpu.VMEM((49 * SLOT, 256), F32),
            pltpu.VMEM((28 * SLOT, 256), F32),
            pltpu.SemaphoreType.DMA((22,)),
            pltpu.SemaphoreType.REGULAR,
        ],
        compiler_params=pltpu.CompilerParams(vmem_limit_bytes=127 * 2**20),
        name="fused_block",
    )(A_x.reshape(S, D), A_wqkv, A_wo, B_w_gate, B_w_up, B_w_down)
    return out.reshape(A_x.shape)
```

```python
import functools
import itertools
import math

import jax
import jax.numpy as jnp
from jax import lax
import jax.experimental.pallas as pl
import jax.experimental.pallas.tpu as pltpu

F32, BF16, U32 = jnp.float32, jnp.bfloat16, jnp.uint32

S, D, F, DH = 2048, 1024, 3584, 32
UNIT = 256
NU = S // UNIT
TQ, CK = 512, 128
NCK = S // CK
TRAIL = NCK + 1
THROTTLE = 4
FC = 512
NFC = F // FC
SLOT = 520
EARLY = 3

_PRODUCTS = (
    (((1, 0, 0), (1, 1, 1)), ((1, 0, 0), (1, 1, 1))),
    (((1, 1, 0), (1, 1, 1)), ((1, 0, 0),)),
    (((1, 0, 0),), ((1, 0, 1), (-1, 1, 1))),
    (((1, 1, 0), (-1, 0, 0)), ((1, 0, 0), (1, 0, 1))),
    (((1, 1, 1),), ((1, 1, 0), (-1, 0, 0))),
    (((1, 0, 0), (1, 0, 1)), ((1, 1, 1),)),
    (((1, 0, 1), (-1, 1, 1)), ((1, 1, 0), (1, 1, 1))),
)
_LHS, _RHS = 0, 1


def _encode(side, levels, get, put, outer=range(7), n=0):
    half = 2 ** (levels - 1)
    for p in outer:
        @functools.cache
        def summed(i, j, terms=_PRODUCTS[p][side]):
            out = get(terms[0][1] * half + i, terms[0][2] * half + j)
            for sign, a, b in terms[1:]:
                out = (lax.add if sign > 0 else lax.sub)(out, get(a * half + i, b * half + j))
            return out

        if levels == 1:
            put(7 * n + p, summed(0, 0))
            yield
            continue
        if levels == 3:
            for i, j in itertools.product(range(4), repeat=2):
                summed(i, j)
                yield
        yield from _encode(side, levels - 1, summed, put, n=7 * n + p)


def _shear(get, by):
    for bit in (1, 2):
        def rows(i, j, get=functools.cache(get), bit=bit):
            return get(i, j) if i & bit else lax.add(get(i, j), lax.mul(get(i | bit, j), by))

        def get(i, j, rows=functools.cache(rows), bit=bit):
            return lax.sub(rows(i, j), lax.mul(rows(i, j ^ bit), by)) if j & bit else rows(i, j)
    return functools.cache(get)


def _encode2(side, get, put):
    get = functools.cache(get)
    sheared = _shear(get, 0.5)
    for fn in (get, sheared):
        for i, j in itertools.product((3, 2, 1, 0), range(4)):
            fn(i, j)
            yield
    yield from _encode(side, 2, sheared, put)


class _Decoder:
    def __init__(self, emit):
        self.emit, self.m = emit, []

    def push(self, v):
        m = self.m
        m.append(v)
        if len(m) == 4:
            self.emit(1, 1, lax.add(lax.add(lax.sub(m[0], m[1]), m[2]), v))
        elif len(m) == 5:
            self.emit(1, 0, lax.add(m[1], v))
            self.t = lax.add(m[0], v)
        elif len(m) == 6:
            self.emit(0, 1, lax.add(m[2], v))
            self.t = lax.sub(self.t, v)
        elif len(m) == 7:
            self.emit(0, 0, lax.add(self.t, v))


def _decode1(product):
    out = {}
    dec = _Decoder(lambda a, b, v: out.update({(a, b): v}))
    for p in range(7):
        dec.push(product(p))
    return out


def _decode2(product, emit):
    sheared = {}
    for i, j in itertools.product(range(2), repeat=2):
        for (a, b), v in _decode1(lambda p: product(4 * p + 2 * i + j)).items():
            sheared[2 * a + i, 2 * b + j] = v
        yield
    get = _shear(lambda i, j: sheared[i, j], -0.5)
    for key in sheared:
        emit(*key, get(*key))
        yield


def _strassen(lhs, rhs, emit):
    dec = _Decoder(emit)
    for q in range(7):
        dec.push(_dot(lhs(q), rhs(q)))
        yield


def _stream(steps):
    return lambda fn: (fn(), steps)


def _chain(*streams):
    return itertools.chain(*[gen for gen, _ in streams]), sum(n for _, n in streams)


def _slowed(stream, every):
    def gen():
        for n, _ in enumerate(stream[0], 1):
            yield
            if n % every == 0:
                yield
    return gen(), stream[1] + stream[1] // every


def _interleave(main, *sides, slack=0):
    done, span = [0] * len(sides), main[1] - slack
    for t in range(main[1]):
        next(main[0])
        for k, (gen, n) in enumerate(sides):
            while done[k] < min(n, -(-n * (t + 1) // span)):
                next(gen)
                done[k] += 1


def _rows(start, size, offset=0):
    first = lax.add(start, offset)
    return pl.ds(first if isinstance(start, int) else pl.multiple_of(first, 8), size)


def _lanes(tile, n=1):
    return slice(tile * 128, (tile + n) * 128)


def _block_row(r):
    return r + (r >> 6) * (UNIT - 64)


def _words(v, dtype=U32):
    return pltpu.bitcast(v.astype(BF16), dtype)


def _from_words(ref, rows, cols=slice(None)):
    return pltpu.bitcast(ref[rows, cols], BF16)


def _stack_halves(v):
    return lax.concatenate([lax.slice_in_dim(v, c, c + 128, axis=1) for c in (0, 128)], 0)


def _dot(a, b):
    return lax.dot_general(a, b, (((1,), (0,)), ((), ())), preferred_element_type=F32)


def _fold_rows(x, reduce):
    while x.size > 8 * x.shape[-1]:
        x = reduce(x.reshape(-1, 2, 8, x.shape[-1]), axis=1)
    return x.reshape(8, -1)


def _start(copies):
    for cp in copies:
        cp.start()


def _wait(copies):
    for cp in copies:
        cp.wait()


def _kernel(x_hbm, wqkv_hbm, wo_hbm, wg_hbm, wu_hbm, wd_hbm, out_hbm,
            x_ref, act_ref, xs_ref, w_ref, ws_ref, wd_ref, wo_ref, h_ref, m_ref, acc_ref, sems, idle_sem):
    zero = pl.semaphore_read(idle_sem)
    regions = itertools.count(1)

    def region(fn):
        n = next(regions)
        pl.when(zero < n)(fn)

    def stage(*streams, **kw):
        region(lambda: _interleave(*streams, **kw))

    def gu_copies(c):
        col = c * FC if isinstance(c, int) else pl.multiple_of(c * FC, FC)
        return [pltpu.make_async_copy(src.at[:, pl.ds(col, FC)], w_ref.at[:, n * FC:(n + 1) * FC], sems.at[n])
                for n, src in enumerate((wg_hbm, wu_hbm))]

    def wd_copy(c):
        row = c * FC if isinstance(c, int) else pl.multiple_of(c * FC, FC)
        return pltpu.make_async_copy(wd_hbm.at[pl.ds(row, FC)], wd_ref, sems.at[2])

    def encode_gu(outer, word_rows=range(0, 64, 8)):
        at = [(t, 2 * t) for t in word_rows]

        @_stream(65 * len(outer) * len(at))
        def stream():
            for t, row in at:
                def get(k, j):
                    tile = j // 2 % 2 * 4 + j // 4 * 2 + j % 2
                    return w_ref[_rows(row, 16, k * 128), _lanes(tile)].astype(F32)

                def put(n, v):
                    ws_ref[_rows(t, 8, n * 64), :] = _words(v)
                yield from _encode(_RHS, 3, get, put, outer)
        return stream

    def gate_up(outer, units=range(NU)):
        @_stream(49 * len(outer) * len(units) // 2)
        def stream():
            for p, pair in itertools.product(range(7 * outer[0], 7 * outer[-1] + 7), zip(units[::2], units[1::2])):
                def lhs(q):
                    return lax.concatenate(
                        [_stack_halves(xs_ref[_rows(((7 * p + q) * NU + u) * 16, 16), :]) for u in pair], 0)

                def emit(a, b, v):
                    for t, u in enumerate(pair):
                        m_ref[_rows(p * SLOT + u * 64 + a * 32, 32), _lanes(b)] = lax.slice_in_dim(
                            v, t * 32, t * 32 + 32)
                yield from _strassen(lhs, lambda q: _from_words(ws_ref, _rows((7 * p + q) * 64, 64)), emit)
        return stream

    def decode_h(starts):
        at = [(r, _block_row(r)) for r in starts]

        @_stream(56 * len(at))
        def stream():
            for (r, row), c in itertools.product(at, range(2)):
                pending = {}

                def emit(i, j, a, b, v):
                    other = pending.pop((a, b, i), None)
                    if other is None:
                        pending[a, b, i] = v
                        return
                    g, u = (other, v) if j else (v, other)
                    h_ref[_rows(row, 8, (2 * a + i) * 64), _lanes(2 * b + c)] = lax.add(u, lax.mul(u, lax.tanh(g)))

                outer = {key: _Decoder(functools.partial(emit, *key))
                         for key in itertools.product(range(2), repeat=2)}
                for p in range(7):
                    for key, v in _decode1(lambda q: m_ref[_rows(r, 8, (7 * p + q) * SLOT), _lanes(c)]).items():
                        outer[key].push(v)
                        yield
        return stream

    def projection_phase(k_ref, qt_ref, vt_ref, wqkv_ref, x2_ref, stat_ref, scale_ref):
        def row_stats(which, first, n_units=1, slot=None):
            base = first * UNIT

            @_stream(n_units * UNIT // 8)
            def stream():
                for r in range(0, n_units * UNIT, 8):
                    rows = _rows(base, 8, r)
                    x = x_ref[rows, :].astype(F32)
                    if which == 0:
                        v = jnp.mean(x, axis=-1, keepdims=True)
                    else:
                        xc = x - lax.concatenate([stat_ref[rows, _lanes(0)]] * 8, 1)
                        v = 0.5 * lax.rsqrt(jnp.mean(xc * xc, axis=-1, keepdims=True) + 1e-5)
                    v = jnp.broadcast_to(v, (8, 128))
                    if slot is None:
                        stat_ref[rows, _lanes(which)] = v
                    else:
                        scale_ref[_rows(slot * UNIT + r, 8), :] = v
                    yield
            return stream

        def normed(row, offset, tile, n, slot=None):
            rows = _rows(row, 8, offset)
            scale = stat_ref[rows, _lanes(1)] if slot is None else scale_ref[_rows(slot * UNIT + offset, 8), :]
            mean, scale = (lax.concatenate([v] * n, 1) for v in (stat_ref[rows, _lanes(0)], scale))
            return lax.mul(lax.sub(x_ref[rows, _lanes(tile, n)].astype(F32), mean), scale)

        def stored(row, offset, tile, n):
            rows = _rows(row + offset, 8)
            return lax.concatenate([act_ref[tile + t, rows, :] for t in range(n)], 1)

        def normalise(u, slot):
            base = u * UNIT

            @_stream(UNIT // 2)
            def stream():
                for r, g in itertools.product(range(0, UNIT, 8), range(0, 8, 2)):
                    v = normed(base, r, g, 2, slot)
                    for t in range(2):
                        act_ref[g + t, _rows(slot * UNIT + r, 8), :] = v[:, _lanes(t)]
                    yield
            return stream

        def encode_x2(slot, xn, row):
            @_stream(8 * 81)
            def stream():
                for r in range(0, 64, 8):
                    def put(n, v):
                        x2_ref[_rows((slot * 49 + n) * 64 + r, 8), :] = v.astype(BF16)
                    yield from _encode2(_LHS, lambda i, k: xn(row, i * 64 + r, 2 * k, 2), put)
            return stream

        def encode_x3(u, xn, row):
            base = u * 16

            @_stream(2 * 7 * 65)
            def stream():
                for r in (0, 8):
                    def get(i, k):
                        return lax.concatenate([xn(row, i * 32 + t + r, k, 1) for t in (0, 16)], 1)

                    def put(n, v):
                        xs_ref[_rows(base, 8, n * NU * 16 + r), :] = v.astype(BF16)
                    yield from _encode(_LHS, 3, get, put)
            return stream

        def encode_qkv(c, word_rows=range(0, 128, 8)):
            @_stream(81 * len(word_rows))
            def stream():
                for t in word_rows:
                    def get(k, j):
                        return wqkv_ref[_rows(k * 256 + 2 * t, 16), _lanes(4 * c + j)].astype(F32)

                    def put(n, v):
                        m_ref[_rows((c // 2 * 49 + n) * 128 + t, 8), _lanes(c % 2)] = _words(v, F32)
                    yield from _encode2(_RHS, get, put)
            return stream

        def product_at(slot, c, n, r, size):
            return _rows(n * SLOT + (slot * 3 + c // 2) * 64 + r, size), _lanes(c % 2)

        def qkv(slots, cols=range(6), outer=range(7)):
            @_stream(7 * len(outer) * len(slots) * len(cols))
            def stream():
                for c, slot, p in itertools.product(cols, slots, outer):
                    def emit(a, b, v):
                        acc_ref[product_at(slot, c, 4 * p + 2 * a + b, 0, 64)] = v
                    yield from _strassen(
                        lambda q: x2_ref[_rows((slot * 49 + 7 * p + q) * 64, 64), :],
                        lambda q: _from_words(m_ref, _rows((c // 2 * 49 + 7 * p + q) * 128, 128), _lanes(c % 2)),
                        emit)
            return stream

        q_scale = 4 * DH ** -0.5 * math.log2(math.e)

        def decode_qkv(slot, cols=range(6)):
            @_stream(8 * 20 * len(cols))
            def stream():
                for c, r in itertools.product(cols, range(0, 64, 8)):
                    def emit(i, j, v):
                        kind, g = divmod(4 * c + j, 8)
                        act_ref[g, _rows((2 + 2 * kind + slot) * UNIT + i * 64 + r, 8), :] = (
                            v if kind else lax.mul(v, q_scale))
                    yield from _decode2(lambda n: acc_ref[product_at(slot, c, n, r, 8)], emit)
            return stream

        def transpose(u, slot):
            q_at, k_at, v_at = (u >> 1) * 512, u * 128, u * 512

            @_stream(48)
            def stream():
                for g, t in itertools.product(range(8), range(2)):
                    get = lambda kind: act_ref[g, _rows((2 + 2 * kind + slot) * UNIT + t * 128, 128), :]
                    qt_ref[_rows(q_at, 64, g * 64), _lanes(2 * slot + t)] = _words(get(0).T)
                    yield
                    k_ref[_rows(k_at, 64, g * S // 2 + t * 64), :] = _words(get(1))
                    yield
                    vt_ref[_rows(v_at, 64, g * 64), _lanes(t)] = _words(get(2).T)
                    yield
            return stream

        @_stream(28 * 12)
        def clear_acc():
            for n, r in itertools.product(range(28), range(0, 384, 32)):
                acc_ref[_rows(n * SLOT + r, 32)] = acc_ref[_rows(n * SLOT + 384 + r % 128, 32)]
                yield

        x_copies = [pltpu.make_async_copy(x_hbm.at[a:b], x_ref.at[a:b], sems.at[3 + n])
                    for n, (a, b) in enumerate(itertools.pairwise((0, UNIT, 2 * UNIT, 4 * UNIT, S)))]
        def w_copy(c, rows, sem):
            return pltpu.make_async_copy(wqkv_hbm.at[rows, _lanes(4 * c, 4)], wqkv_ref.at[rows, _lanes(4 * c, 4)], sem)

        w_copies = {c: w_copy(c, slice(None), sems.at[8 + c]) for c in range(1, 6)}
        first_w = [[w_copy(0, slice(r, r + 128), sems.at[7 + n]) for r in range(n * 128, D, 256)] for n in range(2)]
        _start([x_copies[0], *first_w[0], *first_w[1]])
        for n in range(28):
            acc_ref[n * SLOT + 384:n * SLOT + 512] = jnp.zeros((128, 256), F32)

        x_copies[0].wait()
        _start([x_copies[1], w_copies[1]])
        stage(row_stats(0, 0))
        stage(row_stats(1, 0, slot=0))
        stage(normalise(0, 0))
        _wait(first_w[0])
        stage(encode_x2(0, stored, 0), encode_qkv(0, range(0, 64, 8)))
        _wait(first_w[1])
        stage(encode_qkv(0, range(64, 128, 8)))
        x_copies[1].wait()
        w_copies[2].start()
        stage(row_stats(0, 1))
        stage(qkv([0], [0], range(3)), row_stats(1, 1))
        stage(qkv([0], [0], range(3, 7)), encode_x2(1, normed, UNIT))
        w_copies[1].wait()
        _start([w_copies[3], x_copies[2], w_copies[4], w_copies[5], x_copies[3], *gu_copies(0)])
        stage(qkv([1], [0]), encode_qkv(1))
        stage(qkv([0], [1]), _chain(encode_x3(0, stored, 0), decode_qkv(0, [0])))
        w_copies[2].wait()
        stage(qkv([1], [1]), encode_qkv(2))
        for c, stats in enumerate(([], [row_stats(0, 2, 2)], [row_stats(1, 2)]), 2):
            _wait([w_copies[c + 1]] + x_copies[2:3] * (c == 3))
            stage(qkv([0, 1], [c]), _chain(encode_qkv(c + 1), decode_qkv(0, [c - 1]), *stats))
        x_copies[3].wait()
        stage(qkv([0], [5]), _chain(row_stats(0, 4, 4), row_stats(1, 3, slot=1)), decode_qkv(0, [4]), slack=30)
        stage(qkv([1], [5]), row_stats(1, 4, slot=0),
              _chain(encode_x2(0, normed, 2 * UNIT), normalise(3, 1), decode_qkv(0, [5])))
        _wait(gu_copies(0))

        @pl.loop(1, NU // 2)
        def _(t):
            for slot, other in ((0, 1), (1, 0)):
                u = 2 * t + slot
                ahead = [jnp.minimum(u + n, NU - 1) for n in (1, 2, 3)]
                word = jnp.minimum((u - 2) * 16, 48)
                stage(qkv([slot]), transpose(u - 2, slot), row_stats(1, ahead[2], slot=other),
                      _chain(normalise(ahead[1], slot), encode_x2(other, stored, other * UNIT),
                             encode_x3(ahead[0], stored, other * UNIT), decode_qkv(other),
                             encode_gu(range(EARLY), [word, word + 8])), slack=38)

        wo_copy = pltpu.make_async_copy(wo_hbm, wo_ref, sems.at[3])
        wo_copy.start()
        stage(gate_up(range(EARLY), (0, 3, 4, 5, 6, 7)),
              _chain(*[encode_x3(u, normed, u * UNIT) for u in (1, 2)], encode_gu([EARLY])))
        stage(_chain(gate_up(range(EARLY), (1, 2)), gate_up([EARLY])),
              _chain(encode_gu(range(EARLY + 1, 7)), decode_qkv(1)))
        _start([*gu_copies(1), wd_copy(0)])
        stage(gate_up(range(EARLY + 1, 7)), _chain(transpose(NU - 2, 0), transpose(NU - 1, 1)), clear_acc)
        _wait([*gu_copies(1), wo_copy])

    def attention_phase(k_ref, qt_ref, vt_ref, ot_ref, state_ref, *s_refs):
        def scores(qb, g, j, c):
            q = _from_words(qt_ref, _rows(qb * 512 + g * 64, 16, j * 16))
            q = lax.concatenate([q if i == j else jnp.zeros_like(q) for i in range(4)], 0)
            s = _dot(_from_words(k_ref, _rows(g * (S // 2), CK // 2, c * CK // 2)), q)
            s_refs[j][c * CK:(c + 1) * CK, :] = s
            return _fold_rows(s, jnp.max)

        def values(g, j, c, m):
            p = jnp.exp2(s_refs[j][c * CK:(c + 1) * CK, :] - lax.concatenate([m] * (CK // 8), 0))
            v = _from_words(vt_ref, _rows(g * 64, 16, c // 2 * 512 + j * 16), _lanes(c % 2))
            return _fold_rows(p, jnp.sum), _dot(v, p.astype(BF16))

        def four_heads(it, state, running, do_scores=True, has_prev=True):
            steps = 4 * NCK if do_scores else TRAIL

            @_stream(steps)
            def stream():
                m = {-2: state[0], -1: state[1]}
                acc, l = state[2:]
                place = [((it + back) >> 3, (it + back) & 7) for back in (-1, 0)]
                for t in range(steps):
                    if do_scores:
                        j, c = divmod(t, NCK)
                        part = scores(*place[1], j, c)
                        running.append(part if c == 0 else lax.max(running[-1], part))
                        if c == NCK - 1:
                            m[j] = jnp.broadcast_to(jnp.max(running[-1], axis=0, keepdims=True), (8, TQ))
                    j, c = divmod(t - TRAIL, NCK)
                    if j >= 0 or has_prev:
                        row_max = m[j]
                        if len(running) >= THROTTLE:
                            row_max = row_max + 0.0 * running[-THROTTLE]
                        (qb, g), j = place[j >= 0], j % 4
                        part, o = values(g, j, c, row_max)
                        acc, l = (o, part) if c == 0 else (acc + o, l + part)
                        if c == NCK - 1:
                            ot_ref[j * DH:(j + 1) * DH, :] = acc * (2.0 / jnp.sum(l, axis=0, keepdims=True))
                            if j == 3:
                                act_ref[g, _rows(qb * TQ, TQ), :] = ot_ref[...].T
                    state[:] = [m.get(2), m.get(3), acc, l]
                    yield
            return stream

        spans = list(itertools.pairwise((0, 8, 16, 48, 56)))

        def trip(t, first=False):
            side = _chain(decode_h([t * 32 + r for r in range(0, 32, 8)]), encode_gu(range(EARLY), [(t >> 1) * 8]))

            @region
            def _():
                state, running = [None if first else state_ref[a:b] for a, b in spans], []
                _interleave(_chain(four_heads(2 * t, state, running, has_prev=not first),
                                   four_heads(2 * t + 1, state, running)), side, slack=NCK)
                for (a, b), v in zip(spans, state):
                    state_ref[a:b] = v

        trip(0, first=True)
        pl.loop(1, 16)(trip)
        _interleave(gate_up(range(EARLY)), encode_gu(range(EARLY, 7)),
                    four_heads(32, [state_ref[a:b] for a, b in spans], [], do_scores=False))

    def glu_phase(os_ref, hs_ref, wds_ref, wos_ref):
        def encode_h():
            @_stream(4 * 81 * NU)
            def stream():
                for u, r in itertools.product(range(NU), (0, 8, 32, 40)):
                    def get(i, k):
                        return lax.concatenate(
                            [h_ref[_rows(u * UNIT + i * 64 + r + t, 8), _lanes(k)] for t in (0, 16)], 1)

                    def put(n, v):
                        hs_ref[_rows(n * 256 + u * 32 + r // 32 * 16 + r % 32, 8), :] = v.astype(BF16)
                    yield from _encode2(_LHS, get, put)
            return stream

        def encode_o(starts):
            at = [(r, _block_row(r)) for r in starts]

            @_stream(81 * len(at))
            def stream():
                for r, row in at:
                    def get(i, k):
                        rows = _rows(row, 8, i * 64)
                        return lax.concatenate([act_ref[2 * k + c, rows, :] for c in range(2)], 1)

                    def put(n, v):
                        os_ref[_rows(r, 8, n * 512), :] = v.astype(BF16)
                    yield from _encode2(_LHS, get, put)
            return stream

        def encode_weights(src, dst, column, word_rows):
            depth, at = src.shape[0] // 4, [(t, 2 * t) for t in word_rows]

            @_stream(2 * 81 * len(at))
            def stream():
                for (t, row), c in itertools.product(at, range(2)):
                    def get(k, j):
                        return src[_rows(row, 16, k * depth), _lanes(2 * column(j) + c)].astype(F32)

                    def put(n, v):
                        dst[_rows(t, 8, n * depth // 2), _lanes(c)] = _words(v)
                    yield from _encode2(_RHS, get, put)
            return stream

        def encode_wd():
            return encode_weights(wd_ref, wds_ref, lambda j: 3 - j, range(0, 64, 8))

        def down(r0=0, r1=512):
            @_stream(98 * (r1 - r0) // 32)
            def stream():
                for p, r, c in itertools.product(range(7), range(r0, r1, 32), range(2)):
                    def emit(a, b, v):
                        acc_ref[_rows((4 * p + 2 * a + b) * SLOT + r, 32), _lanes(c)] += v
                    yield from _strassen(
                        lambda q: _stack_halves(hs_ref[_rows((7 * p + q) * 256 + r // 2, 16), :]),
                        lambda q: _from_words(wds_ref, _rows((7 * p + q) * 64, 64), _lanes(c)), emit)
            return stream

        def project(r0, r1, size=32):
            @_stream(98 * (r1 - r0) // size)
            def stream():
                for p, r, c in itertools.product(range(7), range(r0, r1, size), range(2)):
                    def emit(a, b, v):
                        m_ref[_rows((4 * p + 2 * a + b) * SLOT + r, size), _lanes(c)] = v
                    yield from _strassen(
                        lambda q: os_ref[_rows((7 * p + q) * 512 + r, size), :],
                        lambda q: _from_words(wos_ref, _rows((7 * p + q) * 128, 128), _lanes(c)), emit)
            return stream

        def decode_rows(src, emit, r0, r1):
            @_stream(5 * (r1 - r0))
            def stream():
                for r, c in itertools.product(range(r0, r1, 8), range(2)):
                    yield from _decode2(lambda n: src[_rows(n * SLOT + r, 8), _lanes(c)],
                                        lambda i, j, v: emit(_rows(_block_row(r) + i * 64, 8), j, c, v))
            return stream

        def gate(rows, j, c, y):
            half = lax.mul(y, 0.5)
            act_ref[2 * (3 - j) + c, rows, :] = lax.add(half, lax.mul(half, lax.tanh(half)))

        def residual(rows, j, c, s):
            at = rows, _lanes(2 * j + c)
            x_ref[at] = lax.add(x_ref[at].astype(F32), lax.mul(s, act_ref[2 * j + c, rows, :])).astype(BF16)

        @pl.loop(1, NFC)
        def _(c):
            following = gu_copies(jnp.minimum(c + 1, NFC - 1))
            _start(following)
            wd_copy(c - 1).wait()
            word = jnp.minimum((c - 1) * 24, 128 - 24)
            stage(gate_up(range(EARLY, 7)),
                  _chain(encode_h(), encode_wd(),
                         encode_weights(wo_ref, wos_ref, lambda j: j, [word + t for t in (0, 8, 16)])))
            wd_copy(c).start()
            _wait(following)
            stage(down(), _chain(decode_h(range(0, 512, 8)), _slowed(encode_gu(range(EARLY)), 2)))
            row = jnp.minimum((c - 1) * 104, 512 - 104)
            side = _chain(encode_gu(range(EARLY, 7)), encode_o([row + r for r in range(0, 104, 8)]))
            pl.when(c < NFC - 1)(lambda: _interleave(gate_up(range(EARLY)), side))

        out_copies = []

        def write_out(r0, r1):
            for u in range(r0 // 64, -(-r1 // 64)):
                lo, hi = max(r0 - u * 64, 0), min(r1 - u * 64, 64)
                for a, b in [(0, UNIT)] if hi - lo == 64 else [(i + lo, i + hi) for i in range(0, UNIT, 64)]:
                    rows = slice(u * UNIT + a, u * UNIT + b)
                    out_copies.append(pltpu.make_async_copy(x_ref.at[rows], out_hbm.at[rows], sems.at[3]))
                    out_copies[-1].start()

        wd_copy(NFC - 1).wait()
        stage(project(0, 192, 64), _chain(encode_h(), encode_wd()))
        stage(down(0, 192))
        stage(down(192, 512), decode_rows(acc_ref, gate, 0, 192))
        done = 0
        for r0, r1, gated in ((192, 320, (192, 320)), (320, 416, (320, 448)), (416, 480, (448, 512)),
                              (480, 512, (0, 0))):
            stage(project(r0, r1), _chain(decode_rows(m_ref, residual, done, r0), decode_rows(acc_ref, gate, *gated)))
            write_out(done, r0)
            done = r0
        stage(decode_rows(m_ref, residual, done, 512))
        write_out(done, 512)
        _wait(out_copies)

    def attention_block(*kqv):
        pl.run_scoped(
            functools.partial(projection_phase, *kqv),
            pltpu.VMEM((D, 3 * D), BF16),
            pltpu.VMEM((2 * 49 * 64, 256), BF16),
            pltpu.VMEM((S, 256), F32),
            pltpu.VMEM((2 * UNIT, 128), F32),
        )
        pl.run_scoped(
            functools.partial(attention_phase, *kqv),
            pltpu.VMEM((4 * DH, TQ), F32),
            pltpu.VMEM((56, TQ), F32),
            *[pltpu.VMEM((S, TQ), F32)] * 4,
        )

    pl.run_scoped(
        attention_block,
        pltpu.VMEM((8 * S // 2, 128), U32),
        pltpu.VMEM((4 * D // 2, TQ), U32),
        pltpu.VMEM((NU * D // 2, UNIT), U32),
    )
    pl.run_scoped(
        glu_phase,
        pltpu.VMEM((49 * 512, 256), BF16),
        pltpu.VMEM((49 * 256, 256), BF16),
        pltpu.VMEM((49 * 64, 256), U32),
        pltpu.VMEM((49 * 128, 256), U32),
    )


@jax.jit
def pallas_recurrent_scan__softmax_full_mha__glu_gated_glu__prompt_kernel(
    A_x: jax.Array,
    A_wqkv: jax.Array,
    A_wo: jax.Array,
    B_x: jax.Array,
    B_w_gate: jax.Array,
    B_w_up: jax.Array,
    B_w_down: jax.Array,
):
    del B_x
    hbm = pl.BlockSpec(memory_space=pl.ANY)
    out = pl.pallas_call(
        _kernel,
        out_shape=jax.ShapeDtypeStruct((S, D), A_x.dtype),
        in_specs=[hbm] * 6,
        out_specs=hbm,
        scratch_shapes=[
            pltpu.VMEM((S, D), BF16),
            pltpu.VMEM((8, S + 8, 128), F32),
            pltpu.VMEM((343 * NU * 16, 256), BF16),
            pltpu.VMEM((D, 2 * FC), BF16),
            pltpu.VMEM((343 * 64, 128), U32),
            pltpu.VMEM((FC, D), BF16),
            pltpu.VMEM((D, D), BF16),
            pltpu.VMEM((S, FC), F32),
            pltpu.VMEM((49 * SLOT, 256), F32),
            pltpu.VMEM((28 * SLOT, 256), F32),
            pltpu.SemaphoreType.DMA((14,)),
            pltpu.SemaphoreType.REGULAR,
        ],
        compiler_params=pltpu.CompilerParams(vmem_limit_bytes=127 * 2**20),
        name="fused_block",
    )(A_x.reshape(S, D), A_wqkv, A_wo, B_w_gate, B_w_up, B_w_down)
    return out.reshape(A_x.shape)
```
